```python
import os as _os
_os.environ.setdefault("JAX_PLATFORMS", "cpu")
import jax
import jax.numpy as jnp

def _softmax(x, axis=-1):
    return jax.nn.softmax(x, axis=axis)
def _gelu(x):
    return jax.nn.gelu(x, approximate=True)
def _silu(x):
    return jax.nn.silu(x)
def _sigmoid(x):
    return jax.nn.sigmoid(x)
def _layernorm(x, axis=-1, eps=1e-5):
    m = jnp.mean(x, axis=axis, keepdims=True)
    v = jnp.var(x, axis=axis, keepdims=True)
    return (x - m) / jnp.sqrt(v + eps)
def _scatter_add(tgt, idx, src, axis=0):
    return tgt.at[idx].add(src)
def _segment_sum(src, seg, n):
    return jax.ops.segment_sum(src, seg, n)
class _Rng:
    def __init__(self, key):
        self._k = key
    def _next(self):
        self._k, sub = jax.random.split(self._k)
        return sub
    def normal(self, shape):
        return jax.random.normal(self._next(), shape, dtype=jnp.bfloat16)
    def randint(self, lo, hi, shape):
        return jax.random.randint(self._next(), shape, lo, hi, dtype=jnp.int32)
    def uniform(self, shape, lo=0.0, hi=1.0):
        return jax.random.uniform(self._next(), shape, jnp.bfloat16, lo, hi)
    def permutation(self, n):
        return jax.random.permutation(self._next(), n)


kernel_name = 'parallel_sum__sliding_local_dilated__glu_gated_geglu__prompt'

def setup_inputs():
    _rng = _Rng(jax.random.key(int.from_bytes(__import__("os").urandom(4), "little")))
    _w = (lambda a: (lambda t: t.astype(jnp.bfloat16) if jnp.issubdtype(t.dtype, jnp.floating) else t)(jnp.asarray(a)))
    def _A_setup():
        B, S, D = 1, 2048, 512
        return {
            "x": _w((lambda *s: _rng.normal(s) * 0.05)(B, S, D)),
            "wqkv": _w((lambda *s: _rng.normal(s) * 0.05)(D, 3 * D)),
            "wo": _w((lambda *s: _rng.normal(s) * 0.05)(D, D)),
        }
    _A_in = _A_setup()

    def _B_setup():
        B, S, Dm, Df = 1, 2048, 512, 1376
        return {
            "x": _w((lambda *s: _rng.normal(s) * 0.05)(B, S, Dm)),
            "w_gate": _w((lambda *s: _rng.normal(s) * 0.1)(Dm, Df) * (Dm ** -0.5)),
            "w_up": _w((lambda *s: _rng.normal(s) * 0.1)(Dm, Df) * (Dm ** -0.5)),
            "w_down": _w((lambda *s: _rng.normal(s) * 0.1)(Df, Dm) * (Df ** -0.5)),
        }
    _B_in = _B_setup()

    return {
        "A_x": _A_in["x"],
        "A_wqkv": _A_in["wqkv"],
        "A_wo": _A_in["wo"],
        "B_x": _B_in["x"],
        "B_w_gate": _B_in["w_gate"],
        "B_w_up": _B_in["w_up"],
        "B_w_down": _B_in["w_down"],
    }

def reference(A_x, A_wqkv, A_wo, B_x, B_w_gate, B_w_up, B_w_down):
    def _A_ref(x, wqkv, wo):
        B, S, D = x.shape
        H = 32; Dh = D // H
        W, dil = 8, 2
        qkv = (lambda x, *d: x.transpose(*d))((x @ wqkv).reshape(B, S, 3, H, Dh), 2, 0, 3, 1, 4)
        q, k, v = qkv[0], qkv[1], qkv[2]
        scale = Dh ** -0.5
        pos = jnp.arange(S)
        off = jnp.arange(W) * dil
        idx = pos[:, None] - off[None, :]
        mask = idx >= 0
        idx_c = jnp.where(mask, idx, 0).reshape(-1)
        kg = k[:, :, idx_c, :].reshape(B, H, S, W, Dh)
        vg = v[:, :, idx_c, :].reshape(B, H, S, W, Dh)
        logits = jnp.einsum("bhsd,bhswd->bhsw", q, kg) * scale
        logits = jnp.where(mask[None, None, :, :], logits, -1e9)
        attn = _softmax(logits, axis=-1)
        o = jnp.einsum("bhsw,bhswd->bhsd", attn, vg)
        return (lambda x, *d: x.transpose(*d))(o, 0, 2, 1, 3).reshape(B, S, D) @ wo

    def _B_ref(x, w_gate, w_up, w_down):
        g = jnp.einsum("bsd,df->bsf", x, w_gate)
        u = jnp.einsum("bsd,df->bsf", x, w_up)
        h = _gelu(g) * u
        return jnp.einsum("bsf,fd->bsd", h, w_down)

    x = A_x
    xn = _layernorm(x, axis=-1)
    return x + _A_ref(xn, A_wqkv, A_wo) + _B_ref(xn, B_w_gate, B_w_up, B_w_down)
```

```python
import os
import functools
import jax
import jax.numpy as jnp
from jax import lax
import jax.experimental.pallas as pl
import jax.experimental.pallas.tpu as pltpu

S, D, H, DH, W, DIL, DF = 2048, 512, 32, 16, 8, 2, 1376
TM = int(os.environ.get('TM', '512'))
RC = int(os.environ.get('RC', '32'))
USPLIT = int(os.environ.get('USPLIT', '640'))
GP = [int(t) for t in os.environ.get('GP', '384,768,1152').split(',') if t]
OC = int(os.environ.get('OC', '2'))
LNDEP = int(os.environ.get('LNDEP', '1'))
LNMODE = int(os.environ.get('LNMODE', '0'))
HALO = 16
PITCH = 17
NT = (((1,), (1,)), ((), ()))
NSTEP = S // TM
GB = [0] + GP + [DF]
OR = TM // OC


def _gelu_tanh(x):
    c = 0.7978845608028654
    return 0.5 * x * (1.0 + jnp.tanh(c * (x + 0.044715 * (x * x * x))))


def _layernorm_f32(x_bf16):
    x = x_bf16.astype(jnp.float32)
    mean = jnp.mean(x, axis=-1, keepdims=True)
    xc = x - mean
    var = jnp.mean(xc * xc, axis=-1, keepdims=True)
    return xc * lax.rsqrt(var + 1e-5)


def kernel(x_hbm, wqkv_hbm, wo_hbm, wg_hbm, wu_hbm, wd_hbm, out_hbm,
           x_all, out_all, wqkv_raw, t_scr, wqkv_p, wo_raw, wo_p, wg_v, wu_v, wd_v,
           q_scr, k_scr, v_scr, o_scr, xn_scr, sem_x, sem_w, sem_g, sem_o):
    i = pl.program_id(0)

    def x_copy(t):
        return pltpu.make_async_copy(x_hbm.at[pl.ds(t * TM, TM)], x_all.at[pl.ds(t * TM, TM)], sem_x.at[t])

    def out_copy(t):
        r = pl.multiple_of(t * OR, OR)
        return pltpu.make_async_copy(out_all.at[pl.ds(r, OR)], out_hbm.at[pl.ds(r, OR)], sem_o.at[t])

    def g_copy(p):
        return pltpu.make_async_copy(wg_hbm.at[pl.ds(GB[p], GB[p + 1] - GB[p])],
                                     wg_v.at[pl.ds(GB[p], GB[p + 1] - GB[p])], sem_g.at[p])

    cps = {
        'q': pltpu.make_async_copy(wqkv_hbm, wqkv_raw, sem_w.at[0]),
        'u': pltpu.make_async_copy(wu_hbm, wu_v, sem_w.at[1]),
        'd': pltpu.make_async_copy(wd_hbm, wd_v, sem_w.at[2]),
        'o': pltpu.make_async_copy(wo_hbm, wo_raw, sem_w.at[3]),
    }

    def body(first):
        if first:
            x_copy(0).start()
            g_copy(0).start()
            k_scr[:, 0:HALO, :] = jnp.zeros((4, HALO, 128), jnp.float32)
            v_scr[:, 0:HALO, :] = jnp.zeros((4, HALO, 128), jnp.float32)
            x_copy(0).wait()
            for p in range(1, len(GB) - 1):
                g_copy(p).start()
            xn = _layernorm_f32(x_all[0:TM, :]).astype(jnp.bfloat16)
            cur = 0
            row0 = 0
            nxt = TM
        else:
            cur = i % 2
            xn = xn_scr[cur]
            row0 = pl.multiple_of(i * TM, TM)
            nxt = pl.multiple_of(jnp.minimum(i + 1, NSTEP - 1) * TM, TM)
            if LNMODE == 2:
                xn_scr[1 - cur] = _layernorm_f32(x_all[pl.ds(nxt, TM), :]).astype(jnp.bfloat16)

        if first:
            gs = []
            for p in range(len(GB) - 1):
                g_copy(p).wait()
                if p == 0:
                    cps['u'].start()
                elif p == 1:
                    cps['q'].start()
                elif p == 2:
                    x_copy(1).start()
                    cps['d'].start()
                elif p == 3:
                    cps['o'].start()
                gs.append(lax.dot_general(xn, wg_v[GB[p]:GB[p + 1], :], NT,
                                          preferred_element_type=jnp.float32))
            g = jnp.concatenate(gs, axis=1)
        else:
            g = lax.dot_general(xn, wg_v[...], NT, preferred_element_type=jnp.float32)

        if first:
            cps['u'].wait()
            for t in range(2, NSTEP):
                x_copy(t).start()
            u_a = lax.dot_general(xn, wu_v[0:USPLIT, :], NT, preferred_element_type=jnp.float32)
            h_a = (_gelu_tanh(g[:, 0:USPLIT]) * u_a).astype(jnp.bfloat16)
            cps['q'].wait()
            for j in range(12):
                for b in range(4):
                    blk = wqkv_raw[b * 128:(b + 1) * 128, j * 128:(j + 1) * 128].astype(jnp.float32)
                    blkt = blk.T
                    for hl in range(8):
                        t_scr[b, pl.ds((j * 8 + hl) * PITCH, DH), :] = blkt[hl * DH:(hl + 1) * DH, :]
            for m in range(3):
                for b in range(4):
                    for d in range(DH):
                        wqkv_p[m * D + d * H: m * D + (d + 1) * H, b * 128:(b + 1) * 128] = (
                            t_scr[b, pl.ds(m * H * PITCH + d, H, stride=PITCH), :].astype(jnp.bfloat16))
            u_b = lax.dot_general(xn, wu_v[USPLIT:DF, :], NT, preferred_element_type=jnp.float32)
            h_b = (_gelu_tanh(g[:, USPLIT:DF]) * u_b).astype(jnp.bfloat16)
            h = jnp.concatenate([h_a, h_b], axis=1)
            x_copy(1).wait()
            cps['d'].wait()
            cps['o'].wait()
            for b in range(4):
                for hh in range(H):
                    t_scr[b, pl.ds(hh * PITCH, DH), :] = (
                        wo_raw[hh * DH:(hh + 1) * DH, b * 128:(b + 1) * 128].astype(jnp.float32))
            for b in range(4):
                for d in range(DH):
                    wo_p[d * H:(d + 1) * H, b * 128:(b + 1) * 128] = (
                        t_scr[b, pl.ds(d, H, stride=PITCH), :].astype(jnp.bfloat16))

        qkv = lax.dot_general(xn, wqkv_p[...], NT, preferred_element_type=jnp.float32)
        q_scr[...] = qkv[:, 0:D]
        for b in range(4):
            k_scr[b, HALO:HALO + TM, :] = qkv[:, D + b * 128:D + (b + 1) * 128]
            v_scr[b, HALO:HALO + TM, :] = qkv[:, 2 * D + b * 128:2 * D + (b + 1) * 128]

        if not first:
            u = lax.dot_general(xn, wu_v[...], NT, preferred_element_type=jnp.float32)
            h = (_gelu_tanh(g) * u).astype(jnp.bfloat16)

        if LNMODE == 1 or (LNMODE == 2 and first):
            xn_scr[1 - cur] = _layernorm_f32(x_all[pl.ds(nxt, TM), :]).astype(jnp.bfloat16)
        prev = None
        for c in range(TM // RC):
            r0 = c * RC
            if LNMODE == 0:
                xnn = _layernorm_f32(x_all[pl.ds(nxt + r0, RC), :])
                xn_scr[1 - cur, r0:r0 + RC, :] = xnn.astype(jnp.bfloat16)
            bits = None
            if prev is not None:
                bits = pltpu.bitcast(prev, jnp.uint32)
            if LNDEP and LNMODE == 0:
                lb = pltpu.bitcast(xnn[:, 0:128], jnp.uint32)
                bits = lb if bits is None else (bits | lb)
            if bits is not None:
                z = lax.shift_right_logical(lax.shift_right_logical(bits, jnp.uint32(31)), jnp.uint32(1))
                sc = pltpu.bitcast(z + jnp.uint32(0x3e800000), jnp.float32)
                q = q_scr[r0:r0 + RC, :] * jnp.concatenate([sc] * 4, axis=1)
            else:
                q = q_scr[r0:r0 + RC, :] * (DH ** -0.5)
            logits = []
            for w in range(W):
                s = None
                for b in range(4):
                    p = q[:, b * 128:(b + 1) * 128] * k_scr[b, pl.ds(HALO + r0 - DIL * w, RC), :]
                    s = p if s is None else s + p
                s = s + pltpu.roll(s, 64, 1)
                s = s + pltpu.roll(s, 32, 1)
                if first and w > 0 and r0 < DIL * w:
                    row = r0 + lax.broadcasted_iota(jnp.int32, (RC, 128), 0)
                    s = jnp.where(row >= DIL * w, s, -1e9)
                logits.append(s)
            m = logits[0]
            for w in range(1, W):
                m = jnp.maximum(m, logits[w])
            es = [jnp.exp(l - m) for l in logits]
            den = es[0]
            for w in range(1, W):
                den = den + es[w]
            inv = 1.0 / den
            prev = den
            for b in range(4):
                acc = None
                for w in range(W):
                    t = es[w] * v_scr[b, pl.ds(HALO + r0 - DIL * w, RC), :]
                    acc = t if acc is None else acc + t
                o_scr[r0:r0 + RC, b * 128:(b + 1) * 128] = (acc * inv).astype(jnp.bfloat16)

        k_scr[:, 0:HALO, :] = k_scr[:, TM:TM + HALO, :]
        v_scr[:, 0:HALO, :] = v_scr[:, TM:TM + HALO, :]

        b_out = jnp.dot(h, wd_v[...], preferred_element_type=jnp.float32)
        for oc in range(OC):
            r0 = oc * OR
            a_out = jnp.dot(o_scr[r0:r0 + OR, :], wo_p[...], preferred_element_type=jnp.float32)
            rr = row0 + r0 if first else pl.multiple_of(row0 + r0, OR)
            out_all[pl.ds(rr, OR), :] = (
                x_all[pl.ds(rr, OR), :].astype(jnp.float32) + a_out + b_out[r0:r0 + OR, :]
            ).astype(jnp.bfloat16)
            out_copy(oc if first else i * OC + oc).start()
        if first:
            for t in range(2, NSTEP):
                x_copy(t).wait()

    @pl.when(i == 0)
    def _():
        body(True)

    @pl.when(i > 0)
    def _():
        body(False)

    @pl.when(i == NSTEP - 1)
    def _():
        for t in range(NSTEP * OC):
            out_copy(t).wait()


@jax.jit
def pallas_parallel_sum__sliding_local_dilated__glu_gated_geglu__prompt_kernel(
    A_x, A_wqkv, A_wo, B_x, B_w_gate, B_w_up, B_w_down):
    x = A_x.reshape(S, D)
    anyspec = pl.BlockSpec(memory_space=pl.ANY)
    out = pl.pallas_call(
        kernel,
        grid=(NSTEP,),
        in_specs=[anyspec] * 6,
        out_specs=anyspec,
        out_shape=jax.ShapeDtypeStruct((S, D), jnp.bfloat16),
        scratch_shapes=[
            pltpu.VMEM((S, D), jnp.bfloat16),
            pltpu.VMEM((S, D), jnp.bfloat16),
            pltpu.VMEM((D, 3 * D), jnp.bfloat16),
            pltpu.VMEM((4, 3 * H * PITCH + 8, 128), jnp.float32),
            pltpu.VMEM((3 * D, D), jnp.bfloat16),
            pltpu.VMEM((D, D), jnp.bfloat16),
            pltpu.VMEM((D, D), jnp.bfloat16),
            pltpu.VMEM((DF, D), jnp.bfloat16),
            pltpu.VMEM((DF, D), jnp.bfloat16),
            pltpu.VMEM((DF, D), jnp.bfloat16),
            pltpu.VMEM((TM, D), jnp.float32),
            pltpu.VMEM((4, HALO + TM, 128), jnp.float32),
            pltpu.VMEM((4, HALO + TM, 128), jnp.float32),
            pltpu.VMEM((TM, D), jnp.bfloat16),
            pltpu.VMEM((2, TM, D), jnp.bfloat16),
            pltpu.SemaphoreType.DMA((NSTEP,)),
            pltpu.SemaphoreType.DMA((4,)),
            pltpu.SemaphoreType.DMA((len(GB) - 1,)),
            pltpu.SemaphoreType.DMA((NSTEP * OC,)),
        ],
        compiler_params=pltpu.CompilerParams(
            dimension_semantics=("arbitrary",),
            vmem_limit_bytes=100 * 1024 * 1024,
        ),
    )(x, A_wqkv, A_wo, B_w_gate.T, B_w_up.T, B_w_down)
    return out.reshape(1, S, D)
```

```python
import jax
import jax.numpy as jnp
from jax import lax
import jax.experimental.pallas as pl
import jax.experimental.pallas.tpu as pltpu

S, D, H, DH, W, DIL, DF = 2048, 512, 32, 16, 8, 2, 1376
TM = 512
NSTEP = S // TM
RC = 32
HALO = 16
PITCH = 17
USPLIT = 640
GB = (0, 256, 768, DF)
OC = 2
OR = TM // OC
NB = D // 128
NT = (((1,), (1,)), ((), ()))
EPS = 1e-5
NEG = -1e9


def _gelu_tanh(x):
    c = 0.7978845608028654
    return 0.5 * x * (1.0 + jnp.tanh(c * (x + 0.044715 * (x * x * x))))


def _layernorm_f32(x_bf16):
    x = x_bf16.astype(jnp.float32)
    mean = jnp.mean(x, axis=-1, keepdims=True)
    xc = x - mean
    var = jnp.mean(xc * xc, axis=-1, keepdims=True)
    return xc * lax.rsqrt(var + EPS)


def _nt(a, b):
    return lax.dot_general(a, b, NT, preferred_element_type=jnp.float32)


def _kernel(x_hbm, wqkv_hbm, wo_hbm, wg_hbm, wu_hbm, wd_hbm, out_hbm,
            x_all, out_all, wqkv_raw, t_scr, wqkv_p, wo_raw, wo_p, wg_v, wu_v, wd_v,
            q_scr, k_scr, v_scr, o_scr, xn_scr, sem_x, sem_w, sem_g, sem_o):
    i = pl.program_id(0)

    def x_copy(t):
        return pltpu.make_async_copy(
            x_hbm.at[pl.ds(t * TM, TM)], x_all.at[pl.ds(t * TM, TM)], sem_x.at[t])

    def out_copy(t):
        r = pl.multiple_of(t * OR, OR)
        return pltpu.make_async_copy(
            out_all.at[pl.ds(r, OR)], out_hbm.at[pl.ds(r, OR)], sem_o.at[t])

    def g_copy(p):
        n = GB[p + 1] - GB[p]
        return pltpu.make_async_copy(
            wg_hbm.at[pl.ds(GB[p], n)], wg_v.at[pl.ds(GB[p], n)], sem_g.at[p])

    cp_q = pltpu.make_async_copy(wqkv_hbm, wqkv_raw, sem_w.at[0])
    cp_u = pltpu.make_async_copy(wu_hbm, wu_v, sem_w.at[1])
    cp_d = pltpu.make_async_copy(wd_hbm, wd_v, sem_w.at[2])
    cp_o = pltpu.make_async_copy(wo_hbm, wo_raw, sem_w.at[3])

    def body(first):
        if first:
            x_copy(0).start()
            g_copy(0).start()
            k_scr[:, 0:HALO, :] = jnp.zeros((NB, HALO, 128), jnp.float32)
            v_scr[:, 0:HALO, :] = jnp.zeros((NB, HALO, 128), jnp.float32)
            x_copy(0).wait()
            for p in range(1, len(GB) - 1):
                g_copy(p).start()
            xn = _layernorm_f32(x_all[0:TM, :]).astype(jnp.bfloat16)
            cur = 0
            row0 = 0
            nxt = TM

            gs = []
            for p in range(len(GB) - 1):
                g_copy(p).wait()
                if p == 0:
                    cp_u.start()
                elif p == 1:
                    cp_q.start()
                else:
                    x_copy(1).start()
                    cp_d.start()
                    cp_o.start()
                gs.append(_nt(xn, wg_v[GB[p]:GB[p + 1], :]))
            g = jnp.concatenate(gs, axis=1)

            cp_u.wait()
            for t in range(2, NSTEP):
                x_copy(t).start()
            u_a = _nt(xn, wu_v[0:USPLIT, :])
            h_a = (_gelu_tanh(g[:, 0:USPLIT]) * u_a).astype(jnp.bfloat16)

            cp_q.wait()
            for j in range(3 * NB):
                for b in range(NB):
                    blk = wqkv_raw[b * 128:(b + 1) * 128, j * 128:(j + 1) * 128]
                    blkt = blk.astype(jnp.float32).T
                    for hl in range(128 // DH):
                        t_scr[b, pl.ds((j * 8 + hl) * PITCH, DH), :] = blkt[hl * DH:(hl + 1) * DH, :]
            for m in range(3):
                for b in range(NB):
                    for d in range(DH):
                        wqkv_p[m * D + d * H:m * D + (d + 1) * H, b * 128:(b + 1) * 128] = (
                            t_scr[b, pl.ds(m * H * PITCH + d, H, stride=PITCH), :]
                            .astype(jnp.bfloat16))
            u_b = _nt(xn, wu_v[USPLIT:DF, :])
            h_b = (_gelu_tanh(g[:, USPLIT:DF]) * u_b).astype(jnp.bfloat16)
            h = jnp.concatenate([h_a, h_b], axis=1)
        else:
            cur = i % 2
            xn = xn_scr[cur]
            row0 = pl.multiple_of(i * TM, TM)
            nxt = pl.multiple_of(jnp.minimum(i + 1, NSTEP - 1) * TM, TM)

        qkv = _nt(xn, wqkv_p[...])
        q_scr[...] = qkv[:, 0:D]
        for b in range(NB):
            k_scr[b, HALO:HALO + TM, :] = qkv[:, D + b * 128:D + (b + 1) * 128]
            v_scr[b, HALO:HALO + TM, :] = qkv[:, 2 * D + b * 128:2 * D + (b + 1) * 128]

        if first:
            x_copy(1).wait()
            cp_d.wait()
            cp_o.wait()
            for b in range(NB):
                for hh in range(H):
                    t_scr[b, pl.ds(hh * PITCH, DH), :] = (
                        wo_raw[hh * DH:(hh + 1) * DH, b * 128:(b + 1) * 128].astype(jnp.float32))
            for b in range(NB):
                for d in range(DH):
                    wo_p[d * H:(d + 1) * H, b * 128:(b + 1) * 128] = (
                        t_scr[b, pl.ds(d, H, stride=PITCH), :].astype(jnp.bfloat16))
        else:
            g = _nt(xn, wg_v[...])
            u = _nt(xn, wu_v[...])
            h = (_gelu_tanh(g) * u).astype(jnp.bfloat16)

        prev = None
        for c in range(TM // RC):
            r0 = c * RC
            xnn = _layernorm_f32(x_all[pl.ds(nxt + r0, RC), :])
            xn_scr[1 - cur, r0:r0 + RC, :] = xnn.astype(jnp.bfloat16)
            bits = pltpu.bitcast(xnn[:, 0:128], jnp.uint32)
            if prev is not None:
                bits = bits | pltpu.bitcast(prev, jnp.uint32)
            z = lax.shift_right_logical(
                lax.shift_right_logical(bits, jnp.uint32(31)), jnp.uint32(1))
            sc = pltpu.bitcast(z + jnp.uint32(0x3E800000), jnp.float32)

            logits = []
            qs = [q_scr[r0:r0 + RC, b * 128:(b + 1) * 128] * sc for b in range(NB)]
            for w in range(W):
                s = None
                for b in range(NB):
                    p = qs[b] * k_scr[b, pl.ds(HALO + r0 - DIL * w, RC), :]
                    s = p if s is None else s + p
                s = s + pltpu.roll(s, 64, 1)
                s = s + pltpu.roll(s, 32, 1)
                if first and w > 0 and r0 < DIL * w:
                    row = r0 + lax.broadcasted_iota(jnp.int32, (RC, 128), 0)
                    s = jnp.where(row >= DIL * w, s, NEG)
                logits.append(s)
            m = logits[0]
            for w in range(1, W):
                m = jnp.maximum(m, logits[w])
            es = [jnp.exp(l - m) for l in logits]
            den = es[0]
            for w in range(1, W):
                den = den + es[w]
            inv = 1.0 / den
            prev = den
            for b in range(NB):
                acc = None
                for w in range(W):
                    t = es[w] * v_scr[b, pl.ds(HALO + r0 - DIL * w, RC), :]
                    acc = t if acc is None else acc + t
                o_scr[r0:r0 + RC, b * 128:(b + 1) * 128] = (acc * inv).astype(jnp.bfloat16)

        k_scr[:, 0:HALO, :] = k_scr[:, TM:TM + HALO, :]
        v_scr[:, 0:HALO, :] = v_scr[:, TM:TM + HALO, :]

        b_out = jnp.dot(h, wd_v[...], preferred_element_type=jnp.float32)
        for oc in range(OC):
            r0 = oc * OR
            a_out = jnp.dot(o_scr[r0:r0 + OR, :], wo_p[...], preferred_element_type=jnp.float32)
            rr = row0 + r0 if first else pl.multiple_of(row0 + r0, OR)
            out_all[pl.ds(rr, OR), :] = (
                x_all[pl.ds(rr, OR), :].astype(jnp.float32) + a_out + b_out[r0:r0 + OR, :]
            ).astype(jnp.bfloat16)
            out_copy(oc if first else i * OC + oc).start()
        if first:
            for t in range(2, NSTEP):
                x_copy(t).wait()

    @pl.when(i == 0)
    def _():
        body(True)

    @pl.when(i > 0)
    def _():
        body(False)

    @pl.when(i == NSTEP - 1)
    def _():
        for t in range(NSTEP * OC):
            out_copy(t).wait()


@jax.jit
def pallas_parallel_sum__sliding_local_dilated__glu_gated_geglu__prompt_kernel(
    A_x: jax.Array,
    A_wqkv: jax.Array,
    A_wo: jax.Array,
    B_x: jax.Array,
    B_w_gate: jax.Array,
    B_w_up: jax.Array,
    B_w_down: jax.Array,
):
    del B_x
    anyspec = pl.BlockSpec(memory_space=pl.ANY)
    out = pl.pallas_call(
        _kernel,
        grid=(NSTEP,),
        in_specs=[anyspec] * 6,
        out_specs=anyspec,
        out_shape=jax.ShapeDtypeStruct((S, D), jnp.bfloat16),
        scratch_shapes=[
            pltpu.VMEM((S, D), jnp.bfloat16),
            pltpu.VMEM((S, D), jnp.bfloat16),
            pltpu.VMEM((D, 3 * D), jnp.bfloat16),
            pltpu.VMEM((NB, 3 * H * PITCH + 8, 128), jnp.float32),
            pltpu.VMEM((3 * D, D), jnp.bfloat16),
            pltpu.VMEM((D, D), jnp.bfloat16),
            pltpu.VMEM((D, D), jnp.bfloat16),
            pltpu.VMEM((DF, D), jnp.bfloat16),
            pltpu.VMEM((DF, D), jnp.bfloat16),
            pltpu.VMEM((DF, D), jnp.bfloat16),
            pltpu.VMEM((TM, D), jnp.float32),
            pltpu.VMEM((NB, HALO + TM, 128), jnp.float32),
            pltpu.VMEM((NB, HALO + TM, 128), jnp.float32),
            pltpu.VMEM((TM, D), jnp.bfloat16),
            pltpu.VMEM((2, TM, D), jnp.bfloat16),
            pltpu.SemaphoreType.DMA((NSTEP,)),
            pltpu.SemaphoreType.DMA((4,)),
            pltpu.SemaphoreType.DMA((len(GB) - 1,)),
            pltpu.SemaphoreType.DMA((NSTEP * OC,)),
        ],
        compiler_params=pltpu.CompilerParams(
            dimension_semantics=("arbitrary",),
            vmem_limit_bytes=100 * 1024 * 1024,
        ),
    )(A_x.reshape(S, D), A_wqkv, A_wo, B_w_gate.T, B_w_up.T, B_w_down)
    return out.reshape(1, S, D)
```

```python
import jax
import jax.numpy as jnp
from jax import lax
import jax.experimental.pallas as pl
import jax.experimental.pallas.tpu as pltpu

S, D, H, DH, W, DIL, DF = 2048, 512, 32, 16, 8, 2, 1376
TM = 512
NSTEP = S // TM
RC = 32
HALO = 16
PITCH = 17
US1, US2 = 640, 1152
GB = (0, 256, 768, DF)
OC = 2
OR = TM // OC
NB = D // 128
NT = (((1,), (1,)), ((), ()))
EPS = 1e-5
NEG = -1e9


def _gelu_tanh(x):
    c = 0.7978845608028654
    return 0.5 * x * (1.0 + jnp.tanh(c * (x + 0.044715 * (x * x * x))))


def _layernorm_f32(x_bf16, one=None):
    x = x_bf16.astype(jnp.float32)
    if one is not None:
        x = x * jnp.concatenate([one] * NB, axis=1)
    mean = jnp.mean(x, axis=-1, keepdims=True)
    xc = x - mean
    var = jnp.mean(xc * xc, axis=-1, keepdims=True)
    return xc * lax.rsqrt(var + EPS)


def _const_after(bits, const_bits):
    z = lax.shift_right_logical(lax.shift_right_logical(bits, jnp.uint32(31)), jnp.uint32(1))
    return pltpu.bitcast(z + jnp.uint32(const_bits), jnp.float32)


def _nt(a, b):
    return lax.dot_general(a, b, NT, preferred_element_type=jnp.float32)


def _kernel(x_hbm, wqkv_hbm, wo_hbm, wg_hbm, wu_hbm, wd_hbm, out_hbm,
            x_all, out_all, wqkv_raw, t_scr, wqkv_p, wo_raw, wo_p, wg_v, wu_v, wd_v,
            q_scr, k_scr, v_scr, o_scr, xn_scr, sem_x, sem_w, sem_g, sem_o):
    i = pl.program_id(0)

    def x_copy(t):
        return pltpu.make_async_copy(
            x_hbm.at[pl.ds(t * TM, TM)], x_all.at[pl.ds(t * TM, TM)], sem_x.at[t])

    def out_copy(t):
        r = pl.multiple_of(t * OR, OR)
        return pltpu.make_async_copy(
            out_all.at[pl.ds(r, OR)], out_hbm.at[pl.ds(r, OR)], sem_o.at[t])

    def g_copy(p):
        n = GB[p + 1] - GB[p]
        return pltpu.make_async_copy(
            wg_hbm.at[pl.ds(GB[p], n)], wg_v.at[pl.ds(GB[p], n)], sem_g.at[p])

    cp_q = pltpu.make_async_copy(wqkv_hbm, wqkv_raw, sem_w.at[0])
    cp_u = pltpu.make_async_copy(wu_hbm, wu_v, sem_w.at[1])
    cp_d = pltpu.make_async_copy(wd_hbm, wd_v, sem_w.at[2])
    cp_o = pltpu.make_async_copy(wo_hbm, wo_raw, sem_w.at[3])

    def body(first):
        if first:
            x_copy(0).start()
            g_copy(0).start()
            k_scr[:, 0:HALO, :] = jnp.zeros((NB, HALO, 128), jnp.float32)
            v_scr[:, 0:HALO, :] = jnp.zeros((NB, HALO, 128), jnp.float32)
            x_copy(0).wait()
            for p in range(1, len(GB) - 1):
                g_copy(p).start()
            xn = _layernorm_f32(x_all[0:TM, :]).astype(jnp.bfloat16)
            cur = 0
            row0 = 0
            nxt = TM

            gs = []
            for p in range(len(GB) - 1):
                g_copy(p).wait()
                if p == 0:
                    cp_u.start()
                elif p == 1:
                    cp_q.start()
                else:
                    x_copy(1).start()
                    cp_d.start()
                    cp_o.start()
                gs.append(_nt(xn, wg_v[GB[p]:GB[p + 1], :]))
            g = jnp.concatenate(gs, axis=1)

            cp_u.wait()
            for t in range(2, NSTEP):
                x_copy(t).start()
            u_a = _nt(xn, wu_v[0:US1, :])
            h_a = (_gelu_tanh(g[:, 0:US1]) * u_a).astype(jnp.bfloat16)

            cp_q.wait()
            for j in range(3 * NB):
                for b in range(NB):
                    blk = wqkv_raw[b * 128:(b + 1) * 128, j * 128:(j + 1) * 128]
                    blkt = blk.astype(jnp.float32).T
                    for hl in range(128 // DH):
                        t_scr[b, pl.ds((j * 8 + hl) * PITCH, DH), :] = blkt[hl * DH:(hl + 1) * DH, :]
            for m in range(3):
                for b in range(NB):
                    for d in range(DH):
                        wqkv_p[m * D + d * H:m * D + (d + 1) * H, b * 128:(b + 1) * 128] = (
                            t_scr[b, pl.ds(m * H * PITCH + d, H, stride=PITCH), :]
                            .astype(jnp.bfloat16))
            u_b = _nt(xn, wu_v[US1:US2, :])
            h_b = (_gelu_tanh(g[:, US1:US2]) * u_b).astype(jnp.bfloat16)
        else:
            cur = i % 2
            xn = xn_scr[cur]
            row0 = pl.multiple_of(i * TM, TM)
            nxt = pl.multiple_of(jnp.minimum(i + 1, NSTEP - 1) * TM, TM)

        qkv = _nt(xn, wqkv_p[...])
        q_scr[...] = qkv[:, 0:D]
        for b in range(NB):
            k_scr[b, HALO:HALO + TM, :] = qkv[:, D + b * 128:D + (b + 1) * 128]
            v_scr[b, HALO:HALO + TM, :] = qkv[:, 2 * D + b * 128:2 * D + (b + 1) * 128]

        if first:
            x_copy(1).wait()
            cp_d.wait()
            cp_o.wait()
            u_c = _nt(xn, wu_v[US2:DF, :])
            h_c = (_gelu_tanh(g[:, US2:DF]) * u_c).astype(jnp.bfloat16)
            h = jnp.concatenate([h_a, h_b, h_c], axis=1)
            for b in range(NB):
                for hh in range(H):
                    t_scr[b, pl.ds(hh * PITCH, DH), :] = (
                        wo_raw[hh * DH:(hh + 1) * DH, b * 128:(b + 1) * 128].astype(jnp.float32))
            for b in range(NB):
                for d in range(DH):
                    wo_p[d * H:(d + 1) * H, b * 128:(b + 1) * 128] = (
                        t_scr[b, pl.ds(d, H, stride=PITCH), :].astype(jnp.bfloat16))
        else:
            g = _nt(xn, wg_v[...])
            u = _nt(xn, wu_v[...])
            h = (_gelu_tanh(g) * u).astype(jnp.bfloat16)

        prev = None
        for c in range(TM // RC):
            r0 = c * RC
            one = None
            if prev is not None and not first:
                one = _const_after(prev, 0x3F800000)
            xnn = _layernorm_f32(x_all[pl.ds(nxt + r0, RC), :], one)
            xn_scr[1 - cur, r0:r0 + RC, :] = xnn.astype(jnp.bfloat16)
            bits = pltpu.bitcast(xnn[:, 0:128], jnp.uint32)
            if prev is not None:
                bits = bits | prev
            sc = _const_after(bits, 0x3E800000)

            logits = []
            qs = [q_scr[r0:r0 + RC, b * 128:(b + 1) * 128] * sc for b in range(NB)]
            for w in range(W):
                s = None
                for b in range(NB):
                    p = qs[b] * k_scr[b, pl.ds(HALO + r0 - DIL * w, RC), :]
                    s = p if s is None else s + p
                s = s + pltpu.roll(s, 64, 1)
                s = s + pltpu.roll(s, 32, 1)
                if first and w > 0 and r0 < DIL * w:
                    row = r0 + lax.broadcasted_iota(jnp.int32, (RC, 128), 0)
                    s = jnp.where(row >= DIL * w, s, NEG)
                logits.append(s)
            m = logits[0]
            for w in range(1, W):
                m = jnp.maximum(m, logits[w])
            es = [jnp.exp(l - m) for l in logits]
            den = es[0]
            for w in range(1, W):
                den = den + es[w]
            inv = 1.0 / den
            prev = pltpu.bitcast(den, jnp.uint32)
            for b in range(NB):
                acc = None
                for w in range(W):
                    t = es[w] * v_scr[b, pl.ds(HALO + r0 - DIL * w, RC), :]
                    acc = t if acc is None else acc + t
                o_scr[r0:r0 + RC, b * 128:(b + 1) * 128] = (acc * inv).astype(jnp.bfloat16)

        k_scr[:, 0:HALO, :] = k_scr[:, TM:TM + HALO, :]
        v_scr[:, 0:HALO, :] = v_scr[:, TM:TM + HALO, :]

        b_out = jnp.dot(h, wd_v[...], preferred_element_type=jnp.float32)
        for oc in range(OC):
            r0 = oc * OR
            a_out = jnp.dot(o_scr[r0:r0 + OR, :], wo_p[...], preferred_element_type=jnp.float32)
            rr = row0 + r0 if first else pl.multiple_of(row0 + r0, OR)
            out_all[pl.ds(rr, OR), :] = (
                x_all[pl.ds(rr, OR), :].astype(jnp.float32) + a_out + b_out[r0:r0 + OR, :]
            ).astype(jnp.bfloat16)
            out_copy(oc if first else i * OC + oc).start()
        if first:
            for t in range(2, NSTEP):
                x_copy(t).wait()

    @pl.when(i == 0)
    def _():
        body(True)

    @pl.when(i > 0)
    def _():
        body(False)

    @pl.when(i == NSTEP - 1)
    def _():
        for t in range(NSTEP * OC):
            out_copy(t).wait()


@jax.jit
def pallas_parallel_sum__sliding_local_dilated__glu_gated_geglu__prompt_kernel(
    A_x: jax.Array,
    A_wqkv: jax.Array,
    A_wo: jax.Array,
    B_x: jax.Array,
    B_w_gate: jax.Array,
    B_w_up: jax.Array,
    B_w_down: jax.Array,
):
    del B_x
    anyspec = pl.BlockSpec(memory_space=pl.ANY)
    out = pl.pallas_call(
        _kernel,
        grid=(NSTEP,),
        in_specs=[anyspec] * 6,
        out_specs=anyspec,
        out_shape=jax.ShapeDtypeStruct((S, D), jnp.bfloat16),
        scratch_shapes=[
            pltpu.VMEM((S, D), jnp.bfloat16),
            pltpu.VMEM((S, D), jnp.bfloat16),
            pltpu.VMEM((D, 3 * D), jnp.bfloat16),
            pltpu.VMEM((NB, 3 * H * PITCH + 8, 128), jnp.float32),
            pltpu.VMEM((3 * D, D), jnp.bfloat16),
            pltpu.VMEM((D, D), jnp.bfloat16),
            pltpu.VMEM((D, D), jnp.bfloat16),
            pltpu.VMEM((DF, D), jnp.bfloat16),
            pltpu.VMEM((DF, D), jnp.bfloat16),
            pltpu.VMEM((DF, D), jnp.bfloat16),
            pltpu.VMEM((TM, D), jnp.float32),
            pltpu.VMEM((NB, HALO + TM, 128), jnp.float32),
            pltpu.VMEM((NB, HALO + TM, 128), jnp.float32),
            pltpu.VMEM((TM, D), jnp.bfloat16),
            pltpu.VMEM((2, TM, D), jnp.bfloat16),
            pltpu.SemaphoreType.DMA((NSTEP,)),
            pltpu.SemaphoreType.DMA((4,)),
            pltpu.SemaphoreType.DMA((len(GB) - 1,)),
            pltpu.SemaphoreType.DMA((NSTEP * OC,)),
        ],
        compiler_params=pltpu.CompilerParams(
            dimension_semantics=("arbitrary",),
            vmem_limit_bytes=100 * 1024 * 1024,
        ),
    )(A_x.reshape(S, D), A_wqkv, A_wo, B_w_gate.T, B_w_up.T, B_w_down)
    return out.reshape(1, S, D)
```
